```python
import jax
import jax.numpy as jnp

def _softmax(x, axis=-1):
    return jax.nn.softmax(x, axis=axis)
def _gelu(x):
    return jax.nn.gelu(x, approximate=True)
def _silu(x):
    return jax.nn.silu(x)
def _sigmoid(x):
    return jax.nn.sigmoid(x)
def _layernorm(x, axis=-1, eps=1e-5):
    m = jnp.mean(x, axis=axis, keepdims=True)
    v = jnp.var(x, axis=axis, keepdims=True)
    return (x - m) / jnp.sqrt(v + eps)
def _scatter_add(tgt, idx, src, axis=0):
    return tgt.at[idx].add(src)
def _segment_sum(src, seg, n):
    return jax.ops.segment_sum(src, seg, n)
class _Rng:
    def __init__(self, key):
        self._k = key
    def _next(self):
        self._k, sub = jax.random.split(self._k)
        return sub
    def normal(self, shape):
        return jax.random.normal(self._next(), shape, dtype=jnp.bfloat16)
    def randint(self, lo, hi, shape):
        return jax.random.randint(self._next(), shape, lo, hi, dtype=jnp.int32)
    def uniform(self, shape, lo=0.0, hi=1.0):
        return jax.random.uniform(self._next(), shape, jnp.bfloat16, lo, hi)
    def permutation(self, n):
        return jax.random.permutation(self._next(), n)


kernel_name = 'sequential_preLN__sliding_block__glu_gated_glu__prompt'

def _fwd_setup_inputs():
    _rng = _Rng(jax.random.key(int.from_bytes(__import__("os").urandom(4), "little")))
    _w = (lambda a: (lambda t: t.astype(jnp.bfloat16) if jnp.issubdtype(t.dtype, jnp.floating) else t)(jnp.asarray(a)))
    def _A_setup():
        B, S, D = 1, 2048, 512
        return {
            "x": _w((lambda *s: _rng.normal(s) * 0.05)(B, S, D)),
            "wqkv": _w((lambda *s: _rng.normal(s) * 0.05)(D, 3 * D)),
            "wo": _w((lambda *s: _rng.normal(s) * 0.05)(D, D)),
        }
    _A_in = _A_setup()

    def _B_setup():
        B, S, D, F = 1, 2048, 512, 1376
        return {
            "x": _w((lambda *s: _rng.normal(s) * 0.05)(B, S, D)),
            "w_gate": _w((lambda *s: _rng.normal(s) * 0.05)(D, F)),
            "w_up": _w((lambda *s: _rng.normal(s) * 0.05)(D, F)),
            "w_down": _w((lambda *s: _rng.normal(s) * 0.05)(F, D)),
        }
    _B_in = _B_setup()

    return {
        "A_x": _A_in["x"],
        "A_wqkv": _A_in["wqkv"],
        "A_wo": _A_in["wo"],
        "B_x": _B_in["x"],
        "B_w_gate": _B_in["w_gate"],
        "B_w_up": _B_in["w_up"],
        "B_w_down": _B_in["w_down"],
    }

def _fwd_reference(A_x, A_wqkv, A_wo, B_x, B_w_gate, B_w_up, B_w_down):
    def _A_ref(x, wqkv, wo):
        B, S, D = x.shape
        H = 32; Dh = D // H; W = 256
        qkv = (lambda x, *d: x.transpose(*d))((x @ wqkv).reshape(B, S, 3, H, Dh), 2, 0, 3, 1, 4)
        q, k, v = qkv[0], qkv[1], qkv[2]
        scores = jnp.einsum("bhqd,bhkd->bhqk", q, k) * (Dh ** -0.5)
        idx = jnp.arange(S)
        mask = (idx[:, None] - idx[None, :] >= 0) & (idx[:, None] - idx[None, :] < W)
        scores = jnp.where(mask[None, None], scores, -1e9)
        p = _softmax(scores, axis=-1)
        o = jnp.einsum("bhqk,bhkd->bhqd", p, v)
        return (lambda x, *d: x.transpose(*d))(o, 0, 2, 1, 3).reshape(B, S, D) @ wo

    def _B_ref(x, w_gate, w_up, w_down):
        g = jnp.einsum("bsd,df->bsf", x, w_gate)
        u = jnp.einsum("bsd,df->bsf", x, w_up)
        h = _sigmoid(g) * u
        return jnp.einsum("bsf,fd->bsd", h, w_down)

    x = A_x
    h = x + _A_ref(_layernorm(x, axis=-1), A_wqkv, A_wo)
    h2 = h + _B_ref(_layernorm(h, axis=-1), B_w_gate, B_w_up, B_w_down)
    return h2


def setup_inputs():
    _inp = _fwd_setup_inputs()
    _gk = jax.random.fold_in(jax.random.key(int.from_bytes(__import__("os").urandom(4), "little")), 2**31 - 1)
    _shapes = [[1, 2048, 512]]
    _dtypes = ['bfloat16']
    _gks = jax.random.split(_gk, len(_shapes))
    _gs = [jax.random.normal(k, s, dtype=jnp.dtype(d)) * 0.05 for k, s, d in zip(_gks, _shapes, _dtypes)]
    _inp["grad_out"] = _gs[0]
    return _inp

def reference(A_x, A_wqkv, A_wo, B_w_gate, B_w_up, B_w_down, B_x, grad_out):
    _const = dict(B_x=B_x)
    def _f(*_d):
        return _fwd_reference(**{'A_x': _d[0], 'A_wqkv': _d[1], 'A_wo': _d[2], 'B_w_gate': _d[3], 'B_w_up': _d[4], 'B_w_down': _d[5], **_const})
    _out, _vjp = jax.vjp(_f, A_x, A_wqkv, A_wo, B_w_gate, B_w_up, B_w_down)
    _grads = _vjp(grad_out)
    _out0 = jnp.asarray(_out)
    return (_out0, *[jnp.asarray(_g) for _g in _grads])
```

```python
import jax
import jax.numpy as jnp
import jax.experimental.pallas as pl
import jax.experimental.pallas.tpu as pltpu

S, D, F = 2048, 512, 1376
DH, T = 16, 128
NG, HG = 4, 8
NB = S // T
RB = 512
FC = 1376
LOG2E = 1.4426950408889634
f32, bf16 = jnp.float32, jnp.bfloat16


def _nn(a, b):
    return jax.lax.dot_general(a, b, (((1,), (0,)), ((), ())), preferred_element_type=f32)


def _nt(a, b):
    return jax.lax.dot_general(a, b, (((1,), (1,)), ((), ())), preferred_element_type=f32)


def _ln(x):
    c = x - jnp.mean(x, axis=-1, keepdims=True)
    r = 1.0 / jnp.sqrt(jnp.mean(c * c, axis=-1, keepdims=True) + 1e-5)
    return c * r, r


def _ln_bwd(dy, y, r):
    return r * (dy - jnp.mean(dy, axis=-1, keepdims=True)
                - y * jnp.mean(dy * y, axis=-1, keepdims=True))


def _head_weights(t, h):
    parts = [t[h * DH:(h + 1) * DH] if j == h else jnp.zeros((DH, T), bf16) for j in range(HG)]
    return jnp.concatenate(parts, axis=0)


def _kernel(x_h, wqkv_h, wo_h, wg_h, wu_h, wd_h, go_h,
            out_h, dx_h, dwqkv_h, dwo_h, dwg_h, dwu_h, dwd_h,
            x_v, go_v, wqkv_v, wo_v, wg_v, wu_v, wd_v,
            ln1t, qt, kt, vt, kn, vn, ot, p_v, h_v, ln2t, got, hh_v, dg_v, du_v,
            dqt, dkt, dvt, sem):
    ins = [pltpu.make_async_copy(s, d, sem.at[i]) for i, (s, d) in enumerate(
        [(x_h, x_v), (wqkv_h, wqkv_v), (wo_h, wo_v), (wg_h, wg_v), (wu_h, wu_v),
         (go_h, go_v), (wd_h, wd_v)])]
    for c in ins:
        c.start()
    zt = jnp.zeros((NG, 2 * T, T), bf16)
    kn[:, :2 * T] = zt
    vn[:, :2 * T] = zt
    for r in (kt, vt):
        r[:, :2] = jnp.zeros((NG, 2, T, T), bf16)
    ins[0].wait()
    ins[1].wait()

    def qkv_body(i, _):
        rows = pl.ds(pl.multiple_of(i * RB, RB), RB)
        y, _r = _ln(x_v[rows])
        ln1t[:, rows] = y.T.astype(bf16)
        a = _nn(y.astype(bf16), wqkv_v[...])
        for g in range(NG):
            q = a[:, g * T:(g + 1) * T]
            k = a[:, D + g * T:D + (g + 1) * T]
            v = a[:, 2 * D + g * T:2 * D + (g + 1) * T]
            prow = pl.ds(pl.multiple_of(i * RB + 2 * T, T), RB)
            kn[g, prow] = k.astype(bf16)
            vn[g, prow] = v.astype(bf16)
            qT, kT, vT = q.T.astype(bf16), k.T.astype(bf16), v.T.astype(bf16)
            for j in range(RB // T):
                b = i * (RB // T) + j
                qt[g, b] = qT[:, j * T:(j + 1) * T]
                kt[g, b + 2] = kT[:, j * T:(j + 1) * T]
                vt[g, b + 2] = vT[:, j * T:(j + 1) * T]
        return 0
    jax.lax.fori_loop(0, S // RB, qkv_body, 0)

    def tri():
        return (jax.lax.broadcasted_iota(jnp.int32, (T, T), 0)
                > jax.lax.broadcasted_iota(jnp.int32, (T, T), 1))

    def att_body(n, _):
        b, g = n // NG, n % NG
        m = tri()
        k3 = kn[g, pl.ds(pl.multiple_of(b * T, T), 3 * T)]
        q = qt[g, b]
        b0 = jnp.where(b >= 2, 0.0, -1e30)
        b1 = jnp.where(b >= 1, 0.0, -1e30)
        ones = jnp.ones((DH, 3 * T), bf16)
        for h in range(HG):
            hs = slice(h * DH, (h + 1) * DH)
            s = _nn(k3, _head_weights(q, h))
            sa = jnp.where(m, s[:T] + b0, s[2 * T:])
            sb = s[T:2 * T] + b1
            mx = jnp.max(jnp.maximum(sa, sb), axis=0, keepdims=True)
            c = (DH ** -0.5) * LOG2E
            pa = jnp.exp2((sa - mx) * c).astype(bf16)
            pb = jnp.exp2((sb - mx) * c).astype(bf16)
            p_v[n, h, :T] = pa
            p_v[n, h, T:] = pb
            z = jnp.zeros_like(pa)
            p3 = jnp.concatenate([jnp.where(m, pa, z), pb, jnp.where(m, z, pa)], axis=0)
            v3 = jnp.concatenate([vt[g, b + j, hs] for j in range(3)], axis=1)
            o = _nn(jnp.concatenate([v3, ones], axis=0), p3)
            inv = 1.0 / o[DH:DH + 1]
            ot[g, b, hs] = (o[:DH] * inv).astype(bf16)
            dqt[g, b, h:h + 1] = inv
        return 0
    jax.lax.fori_loop(0, NB * NG, att_body, 0)

    for c in ins[2:]:
        c.wait()

    R2 = 256
    def ffn_body(i, _):
        rows = pl.ds(pl.multiple_of(i * R2, R2), R2)
        oT = jnp.concatenate([jnp.concatenate(
            [ot[g, i * (R2 // T) + j] for j in range(R2 // T)], axis=1) for g in range(NG)], axis=0)
        h = x_v[rows].astype(f32) + _nn(oT.astype(f32).T.astype(bf16), wo_v[...])
        y, r = _ln(h)
        yb = y.astype(bf16)
        ln2t[:, rows] = y.T.astype(bf16)
        go = go_v[rows]
        got[:, rows] = go.astype(f32).T.astype(bf16)
        gt = _nn(yb, wg_v[...])
        u = _nn(yb, wu_v[...])
        sg = 1.0 / (1.0 + jnp.exp(-gt))
        hh = sg * u
        hb = hh.astype(bf16)
        hh_v[rows] = hb
        x_v[rows] = (h + _nn(hb, wd_v[...])).astype(bf16)
        dhh = _nt(go, wd_v[...])
        du = dhh * sg
        dg = du * (u - hh)
        dub, dgb = du.astype(bf16), dg.astype(bf16)
        du_v[rows] = dub
        dg_v[rows] = dgb
        dy = _nt(dgb, wg_v[...]) + _nt(dub, wu_v[...])
        h_v[rows] = go.astype(f32) + _ln_bwd(dy, y, r)
        return 0
    jax.lax.fori_loop(0, S // R2, ffn_body, 0)
    outs = [pltpu.make_async_copy(s, d, sem.at[i]) for i, (s, d) in enumerate(
        [(x_v, out_h), (go_v, dx_h), (wqkv_v, dwqkv_h), (wo_v, dwo_h), (wg_v, dwg_h),
         (wu_v, dwu_h), (wd_v, dwd_h)])]
    outs[0].start()

    wg_v[...] = _nn(ln2t[...], dg_v[...]).astype(bf16)
    outs[4].start()
    wu_v[...] = _nn(ln2t[...], du_v[...]).astype(bf16)
    outs[5].start()
    wd_v[...] = _nn(got[...], hh_v[...]).T.astype(bf16)
    outs[6].start()

    dhb = h_v[...].astype(bf16)
    got[...] = _nt(wo_v[...], dhb).astype(bf16)
    oT = jnp.concatenate([jnp.concatenate(
        [ot[g, j] for j in range(NB)], axis=1) for g in range(NG)], axis=0)
    wo_v[...] = _nn(oT, dhb).astype(bf16)
    outs[3].start()

    def bwd(acc_k, acc_v):
        acc_k[:, :2] = jnp.zeros((2, 2, T, D), f32).reshape(2, 2, T, D)
        acc_v[:, :2] = jnp.zeros((2, 2, T, D), f32).reshape(2, 2, T, D)

    def att_bwd(n, _):
        b, g = n // NG, n % NG
        m = tri()
        v3 = vn[g, pl.ds(pl.multiple_of(b * T, T), 3 * T)]
        grow = pl.ds(pl.multiple_of(g * T, T), T)
        do = got[grow, pl.ds(pl.multiple_of(b * T, T), T)]
        dof, o, q = do.astype(f32), ot[g, b].astype(f32), qt[g, b]
        invs = dqt[g, b, :HG]
        dqs, dks, dvs = [], [], []
        for h in range(HG):
            hs = slice(h * DH, (h + 1) * DH)
            inv = invs[h:h + 1]
            dos = (dof[hs] * inv).astype(bf16)
            delta = jnp.sum(dos.astype(f32) * o[hs], axis=0, keepdims=True)
            dp = _nn(v3, _head_weights(jnp.concatenate([dos] * HG, axis=0), h))
            pa, pb = p_v[n, h, :T], p_v[n, h, T:]
            da = (pa.astype(f32) * (jnp.where(m, dp[:T], dp[2 * T:]) - delta)).astype(bf16)
            db = (pb.astype(f32) * (dp[T:2 * T] - delta)).astype(bf16)
            z = jnp.zeros_like(pa)
            p3 = jnp.concatenate([jnp.where(m, pa, z), pb, jnp.where(m, z, pa)], axis=0)
            d3 = jnp.concatenate([jnp.where(m, da, z), db, jnp.where(m, z, da)], axis=0)
            k3 = jnp.concatenate([kt[g, b + j, hs] for j in range(3)], axis=1)
            dqs.append(_nn(k3, d3))
            dks.append(_nt(q[hs], d3))
            dvs.append(_nt(dos, p3))
        sc = DH ** -0.5
        dqt[g, b] = jnp.concatenate(dqs, axis=0) * sc
        dk = jnp.concatenate(dks, axis=0) * sc
        dv = jnp.concatenate(dvs, axis=0)
        for j in range(2):
            dkt[g, b + j] += dk[:, j * T:(j + 1) * T]
            dvt[g, b + j] += dv[:, j * T:(j + 1) * T]
        dkt[g, b + 2] = dk[:, 2 * T:]
        dvt[g, b + 2] = dv[:, 2 * T:]
        return 0
    dkt[:, :2] = jnp.zeros((NG, 2, T, T), f32)
    dvt[:, :2] = jnp.zeros((NG, 2, T, T), f32)
    jax.lax.fori_loop(0, NB * NG, att_bwd, 0)

    outs[0].wait()
    xin = pltpu.make_async_copy(x_h, x_v, sem.at[7])
    xin.start()

    def blk(j):
        return jnp.concatenate(
            [dqt[g, j] for g in range(NG)] + [dkt[g, j + 2] for g in range(NG)]
            + [dvt[g, j + 2] for g in range(NG)], axis=0).astype(bf16)
    xin.wait()

    def dx_body(i, _):
        rows = pl.ds(pl.multiple_of(i * RB, RB), RB)
        dT = jnp.concatenate([blk(i * (RB // T) + j) for j in range(RB // T)], axis=1)
        dy = _nn(wqkv_v[...], dT).T
        y, r = _ln(x_v[rows])
        go_v[rows] = (h_v[rows] + _ln_bwd(dy, y, r)).astype(bf16)
        return 0
    jax.lax.fori_loop(0, S // RB, dx_body, 0)
    outs[1].start()
    for t in range(3):
        src, off = ((dqt, 0), (dkt, 2), (dvt, 2))[t]
        dT = jnp.concatenate([jnp.concatenate(
            [src[g, j + off] for j in range(NB)], axis=1) for g in range(NG)], axis=0).astype(bf16)
        wqkv_v[:, t * D:(t + 1) * D] = _nt(ln1t[...], dT).astype(bf16)
    outs[2].start()
    for c in outs[1:]:
        c.wait()


@jax.jit
def pallas_sequential_preLN__sliding_block__glu_gated_glu__prompt_kernel(
    A_x, A_wqkv, A_wo, B_x, B_w_gate, B_w_up, B_w_down, grad_out,
):
    V = pltpu.VMEM
    sds = jax.ShapeDtypeStruct
    outs = pl.pallas_call(
        _kernel,
        in_specs=[pl.BlockSpec(memory_space=pl.ANY)] * 7,
        out_specs=[pl.BlockSpec(memory_space=pl.ANY)] * 7,
        out_shape=[sds((S, D), bf16), sds((S, D), bf16), sds((D, 3 * D), bf16), sds((D, D), bf16),
                   sds((D, F), bf16), sds((D, F), bf16), sds((F, D), bf16)],
        scratch_shapes=[
            V((S, D), bf16), V((S, D), bf16), V((D, 3 * D), bf16), V((D, D), bf16),
            V((D, F), bf16), V((D, F), bf16), V((F, D), bf16),
            V((D, S), bf16), V((NG, NB, T, T), bf16), V((NG, NB + 2, T, T), bf16),
            V((NG, NB + 2, T, T), bf16), V((NG, S + 2 * T, T), bf16), V((NG, S + 2 * T, T), bf16),
            V((NG, NB, T, T), bf16), V((NB * NG, HG, 2 * T, T), bf16), V((S, D), f32),
            V((D, S), bf16), V((D, S), bf16), V((S, F), bf16), V((S, F), bf16), V((S, F), bf16),
            V((NG, NB, T, T), f32), V((NG, NB + 2, T, T), f32), V((NG, NB + 2, T, T), f32),
            pltpu.SemaphoreType.DMA((8,)),
        ],
        compiler_params=pltpu.CompilerParams(vmem_limit_bytes=127 * 2**20),
    )(A_x.reshape(S, D), A_wqkv, A_wo, B_w_gate, B_w_up, B_w_down, grad_out.reshape(S, D))
    return (outs[0].reshape(1, S, D), outs[1].reshape(1, S, D), *outs[2:])
```

```python
import functools

import jax
import jax.numpy as jnp
import jax.experimental.pallas as pl
import jax.experimental.pallas.tpu as pltpu

S, D, F = 2048, 512, 1376
DH, T = 16, 128
HT = T // 2
NG, HG = 4, 8
NB = S // T
RB = 512
LOG2E = 1.4426950408889634
f32, bf16 = jnp.float32, jnp.bfloat16


def _nn(a, b):
    return jax.lax.dot_general(a, b, (((1,), (0,)), ((), ())), preferred_element_type=f32)


def _nt(a, b):
    return jax.lax.dot_general(a, b, (((1,), (1,)), ((), ())), preferred_element_type=f32)


def _ln(x):
    c = x - jnp.mean(x, axis=-1, keepdims=True)
    r = 1.0 / jnp.sqrt(jnp.mean(c * c, axis=-1, keepdims=True) + 1e-5)
    return c * r, r


def _ln_bwd(dy, y, r):
    return r * (dy - jnp.mean(dy, axis=-1, keepdims=True)
                - y * jnp.mean(dy * y, axis=-1, keepdims=True))


def _and(t, m):
    return pltpu.bitcast(pltpu.bitcast(t, jnp.uint32) & m, bf16)


def _split(e, m):
    u = pltpu.bitcast(e, jnp.uint32)
    lo = u & m
    return pltpu.bitcast(lo, bf16), pltpu.bitcast(u ^ lo, bf16)


def _packed_mask(cond):
    w = pltpu.bitcast(jnp.where(cond, 1.0, 0.0).astype(bf16), jnp.uint32)
    return ((w >> 7) & 0x10001) * 0xFFFF


def _iota(shape, axis):
    return jax.lax.broadcasted_iota(jnp.int32, shape, axis)


def _halves(t, e, msk):
    lo, hi = msk[HG, :DH // 2], msk[HG + 1, :DH // 2]
    m0, m1 = (lo, hi) if e == 0 else (hi, lo)
    return jnp.concatenate([_and(t[:DH], m0), _and(t[DH:], m1)], axis=0)


def _pair_rows(a, b):
    lo = _iota((DH, T), 1) < HT
    return jnp.concatenate([jnp.where(lo, a[:DH], b[:DH]),
                            pltpu.roll(jnp.where(lo, b[DH:], a[DH:]), HT, 1)], axis=0)


def _rot_odd(t):
    return jnp.concatenate([pltpu.roll(t[h * DH:(h + 1) * DH], HT, 1) if h % 2
                            else t[h * DH:(h + 1) * DH] for h in range(HG)], axis=0)


def _kernel(x_h, wqkv_h, wo_h, wg_h, wu_h, wd_h, go_h,
            out_h, dx_h, dwqkv_h, dwo_h, dwg_h, dwu_h, dwd_h,
            x_v, go_v, wqkv_v, wo_v, wg_v, wu_v, wd_v,
            ln1t, qt, qr, kt, vt, kn, ot, inv_v, p_v, h_v, ln2t, got, hh_v, dg_v, du_v,
            dqkv, acc_v, s_v, mx_v, do_v, s2_v, dn_v, m64_v, mab_v, mt_v, msk, sem):
    ins = [pltpu.make_async_copy(s, d, sem.at[i]) for i, (s, d) in enumerate(
        [(x_h.at[:RB], x_v.at[:RB]), (wqkv_h.at[:, :D], wqkv_v.at[:, :D]), (wo_h, wo_v), (wg_h, wg_v), (wu_h, wu_v),
         (go_h, go_v), (wd_h, wd_v), (x_h.at[RB:], x_v.at[RB:]),
         (wqkv_h.at[:, D:2 * D], wqkv_v.at[:, D:2 * D]), (wqkv_h.at[:, 2 * D:], wqkv_v.at[:, 2 * D:])])]
    ins[0].start()
    ins[1].start()
    ins[8].start()
    zt = jnp.zeros((NG, 2 * T, T), bf16)
    kn[:, :2 * T] = zt
    for r in (kt, vt):
        r[:, :2] = jnp.zeros((NG, 2, T, T), bf16)
    m64_v[...] = _packed_mask(_iota((HT, T), 0) > _iota((HT, T), 1) % HT)
    mab_v[...] = _packed_mask(_iota((T, T), 1) > _iota((T, T), 0))
    mt_v[...] = _packed_mask(_iota((T, T), 0) > _iota((T, T), 1))
    c_ = _iota((HT, T), 1)
    for j in range(HG):
        msk[j] = _packed_mask(c_ // DH == j)
    msk[HG] = _packed_mask(c_ < HT)
    msk[HG + 1] = _packed_mask(c_ >= HT)
    ins[0].wait()

    def qkv_body(i, _, first=False):
        rows = pl.ds(pl.multiple_of(i * RB, RB), RB)
        y, _r = _ln(x_v[rows].astype(f32))
        yb = y.astype(bf16)
        ln1t[:, rows] = yb.T
        if first:
            parts = []
            for t, (now, nxt) in enumerate(((1, [9]), (8, [7]), (9, [2, 3, 4, 5, 6]))):
                ins[now].wait()
                for j in nxt:
                    ins[j].start()
                parts.append(_nn(yb, wqkv_v[:, t * D:(t + 1) * D]))
            a = jnp.concatenate(parts, axis=1)
        else:
            a = _nn(yb, wqkv_v[...])
        for g in range(NG):
            q = a[:, g * T:(g + 1) * T] * ((DH ** -0.5) * LOG2E)
            k = a[:, D + g * T:D + (g + 1) * T].astype(bf16)
            v = a[:, 2 * D + g * T:2 * D + (g + 1) * T].astype(bf16)
            kn[g, pl.ds(pl.multiple_of(i * RB + 2 * T, T), RB)] = k
            qT, kT, vT = q.T, k.T, v.T
            for j in range(RB // T):
                b = i * (RB // T) + j
                qt[g, b] = qT[:, j * T:(j + 1) * T].astype(bf16)
                qr[g, b] = _rot_odd(qT[:, j * T:(j + 1) * T]).astype(bf16)
                kt[g, b + 2] = kT[:, j * T:(j + 1) * T]
                vt[g, b + 2] = vT[:, j * T:(j + 1) * T]
        return 0
    qkv_body(0, 0, True)

    last = NB * NG - 1

    def scores(n, u, edge):
        b, g = n // NG, n % NG
        p, e = divmod(u, 2)
        k = kn[g, pl.ds(pl.multiple_of(b * T + e * HT, HT), 2 * T + HT)]
        w = _halves(qr[g, b, p * 2 * DH:(p + 1) * 2 * DH], e, msk)
        w = jnp.concatenate([w if j == p else jnp.zeros((2 * DH, T), bf16)
                             for j in range(HG // 2)], axis=0)
        s = _nn(k, w)
        n0 = T - e * HT
        s0, s1, s2 = s[:n0], s[n0:n0 + T], s[n0 + T:]
        if edge:
            s0 = s0 + jnp.where(b >= 2, 0.0, -1e30)
            s1 = s1 + jnp.where(b >= 1, 0.0, -1e30)
        tri = _iota((HT, T), 0) > _iota((HT, T), 1) % HT
        if e == 0:
            xa, xb = jnp.where(tri, s0[:HT], s2), s0[HT:]
        else:
            xa, xb = s2[:HT], jnp.where(tri, s0, s2[HT:])
        s_v[u, :HT] = xa
        s_v[u, HT:T] = xb
        s_v[u, T:] = s1
        mx_v[u] = jnp.max(jnp.maximum(jnp.maximum(xa, xb), jnp.maximum(s1[:HT], s1[HT:])),
                          axis=0, keepdims=True)

    def key_rows(x, y, e):
        z = jnp.zeros((HT, T), bf16)
        lo, hi = _split(x[:HT] if e == 0 else x[HT:], m64_v[...])
        parts = [lo, x[HT:], y, hi, z] if e == 0 else [z, lo, y, x[:HT], hi]
        return jnp.concatenate(parts, axis=0)

    for u in range(HG - 1):
        scores(0, u, True)
    ins[7].wait()
    jax.lax.fori_loop(1, S // RB, qkv_body, 0, unroll=3)

    def att_body(n, _, edge):
        b, g = n // NG, n % NG
        scores(n, HG - 1, edge)
        for u in range(HG):
            p, e = divmod(u, 2)
            ps = slice(p * 2 * DH, (p + 1) * 2 * DH)
            s = s_v[u]
            e32 = jnp.exp2(s - mx_v[u])
            inv = 1.0 / jnp.sum(e32, axis=0, keepdims=True)
            pr = e32.astype(bf16)
            for c in (slice(0, T), slice(T, 2 * T)):
                pt = e32[c].T.astype(bf16)
                p_v[n, 2 * p + e, e * HT:(e + 1) * HT, c] = pt[:HT]
                p_v[n, 2 * p + 1 - e, e * HT:(e + 1) * HT, c] = pt[HT:]
            v3 = jnp.concatenate([vt[g, b + j, ps] for j in range(3)], axis=1)
            o = _nn(v3, key_rows(pr[:T], pr[T:], e)) * inv
            if e == 0:
                oa, inva = o, inv
            else:
                ot[g, b, ps] = _pair_rows(oa, o).astype(bf16)
                it = _pair_rows(jnp.broadcast_to(inva, (2 * DH, T)), jnp.broadcast_to(inv, (2 * DH, T)))
                inv_v[g, b, 2 * p:2 * p + 1] = it[:1]
                inv_v[g, b, 2 * p + 1:2 * p + 2] = it[DH:DH + 1]
            if u:
                scores(jnp.minimum(n + 1, last), u - 1, edge)
        return 0
    jax.lax.fori_loop(0, NB * NG, functools.partial(att_body, edge=True), 0, unroll=16)

    for c in ins[2:7]:
        c.wait()

    R2 = 256
    def ffn_body(i, _):
        rows = pl.ds(pl.multiple_of(i * R2, R2), R2)
        oT = jnp.concatenate([jnp.concatenate(
            [ot[g, i * (R2 // T) + j] for j in range(R2 // T)], axis=1) for g in range(NG)], axis=0)
        h = x_v[rows].astype(f32) + _nn(oT.T, wo_v[...])
        go = go_v[rows]
        dhh = _nt(go, wd_v[...])
        y, r = _ln(h)
        yb = y.astype(bf16)
        go = go_v[rows]
        got[:, rows] = go.T
        gt = _nt(yb, wg_v[...])
        u = _nt(yb, wu_v[...])
        ln2t[:, rows] = yb.T
        sg = 1.0 / (1.0 + jnp.exp(-gt))
        hh = sg * u
        hb = hh.astype(bf16)
        hh_v[rows] = hb
        du = dhh * sg
        dg = du * (u - hh)
        dub, dgb = du.astype(bf16), dg.astype(bf16)
        du_v[rows] = dub
        dg_v[rows] = dgb
        dy = _nn(dgb, wg_v[...]) + _nn(dub, wu_v[...])
        x_v[rows] = (h + _nn(hb, wd_v[...])).astype(bf16)
        h_v[rows] = go.astype(f32) + _ln_bwd(dy, y, r)
        return 0
    jax.lax.fori_loop(0, S // R2, ffn_body, 0, unroll=2)
    outs = [pltpu.make_async_copy(s, d, sem.at[i]) for i, (s, d) in enumerate(
        [(x_v, out_h), (go_v, dx_h), (wo_v, dwo_h), (wg_v, dwg_h),
         (wu_v, dwu_h), (wd_v, dwd_h)])]
    outs[0].start()

    wg_v[...] = _nn(ln2t[...], dg_v[...]).T.astype(bf16)
    outs[3].start()
    wu_v[...] = _nn(ln2t[...], du_v[...]).T.astype(bf16)
    outs[4].start()
    wd_v[...] = _nn(got[...], hh_v[...]).T.astype(bf16)
    outs[5].start()

    dhb = h_v[...].astype(bf16)
    got[...] = _nt(wo_v[...], dhb).astype(bf16)

    def dscores(n, slot):
        b, g = n // NG, n % NG
        do = got[pl.ds(pl.multiple_of(g * T, T), T), pl.ds(pl.multiple_of(b * T, T), T)]
        do, o, invs = do.astype(f32), ot[g, b].astype(f32), inv_v[g, b]
        row = jax.lax.broadcasted_iota(jnp.int32, (DH, T), 0)
        dos, das, dbs = [], [], []
        for h in range(HG):
            hs = slice(h * DH, (h + 1) * DH)
            d = (do[hs] * invs[h:h + 1]).astype(bf16).astype(f32)
            nd = -jnp.sum(d * o[hs], axis=0, keepdims=True)
            hi = nd.astype(bf16).astype(f32)
            dos.append(d.astype(bf16))
            for dst, r0 in ((das, 0), (dbs, 2)):
                dst.append(jnp.where(row == r0, hi, jnp.where(row == r0 + 1, nd - hi, 0.0)).astype(bf16))
        dall = jnp.concatenate(dos, axis=0)
        do_v[slot] = dall
        dn_v[0] = dall.T
        dn_v[1] = jnp.concatenate([das[h ^ 1] for h in range(HG)], axis=0).T
        dn_v[2] = jnp.concatenate([dos[h ^ 2] for h in range(HG)], axis=0).T
        dn_v[3] = jnp.concatenate([dbs[h ^ 1] for h in range(HG)], axis=0).T

    def dheads(n):
        b, g = n // NG, n % NG
        ones = jnp.ones((DH, T), bf16)
        zero = jnp.zeros((DH, T), bf16)
        row, lane = _iota((DH, T), 0), _iota((DH, T), 1)
        edge_ones = jnp.where(((row < 2) & (lane < HT)) | ((row // 2 == 1) & (lane >= HT)),
                              1.0, 0.0).astype(bf16)

        def bits(k, rows, slot):
            return pltpu.bitcast(dn_v[k, rows], jnp.uint32) & msk[slot]

        def head(h):
            hs = slice(h * DH, (h + 1) * DH)
            ra, rb = slice(0, HT), slice(HT, T)
            la = bits(0, ra, h) | bits(1, ra, h ^ 1)
            lb = bits(0, rb, h) | bits(1, rb, h ^ 1)
            lh = la | bits(2, rb, h ^ 2) | bits(3, rb, h ^ 1)
            la, lb, lh = (pltpu.bitcast(t, bf16) for t in (la, lb, lh))

            def w(j):
                t = vt[g, b + j]
                return jnp.concatenate([ones if k == (h ^ 1) else t[k * DH:(k + 1) * DH]
                                        for k in range(HG)], axis=0)
            blocks = {h: _and(vt[g, b + 2, hs], msk[HG, :DH // 2]),
                      h ^ 2: _and(vt[g, b, hs], msk[HG + 1, :DH // 2]), h ^ 1: edge_ones}
            wh = jnp.concatenate([blocks.get(k, zero) for k in range(HG)], axis=0)
            dh = _nn(lh, wh)
            tri = _iota((HT, T), 1) > _iota((HT, T), 0)
            s2_v[h, ra, :T] = jnp.where(tri, _nn(la, w(0)), dh)
            tri = _iota((HT, T), 1) > _iota((HT, T), 0) + HT
            s2_v[h, rb, :T] = jnp.where(tri, dh, _nn(lb, w(2)))
            s2_v[h, :, T:] = _nn(jnp.concatenate([la, lb], axis=0), w(1))
        return head

    dscores(0, 0)
    head0 = dheads(0)
    for h in range(HG):
        head0(h)
    dscores(1, 1)
    oT = jnp.concatenate([jnp.concatenate(
        [ot[g, j] for j in range(NB)], axis=1) for g in range(NG)], axis=0)
    wo_v[...] = _nn(oT, dhb).astype(bf16)
    outs[2].start()


    def att_bwd(n, _):
        b, g = n // NG, n % NG
        dqs, dks, dvs = [], [], []
        dall = do_v[n % 2]
        head = dheads(jnp.minimum(n + 1, last))
        z = jnp.zeros((HT, T), bf16)
        for h in range(HG):
            hs = slice(h * DH, (h + 1) * DH)
            pr = p_v[n, h]
            d = (pr.astype(f32) * s2_v[h]).astype(bf16)
            p0, p2 = _split(pr[:, :T], mab_v[...])
            dvs.append(_nn(dall[hs], jnp.concatenate([p0, pr[:, T:], p2], axis=1)))
            k3 = jnp.concatenate([kt[g, b + j, hs] for j in range(3)], axis=1)
            d0, d2 = _split(d[:, :T], mab_v[...])
            t0, t2 = _split(d[:, :T].T, mt_v[...])
            dqs.append(_nn(k3, jnp.concatenate([t0, d[:, T:].T, t2], axis=0)))
            dks.append(_nn(qt[g, b, hs], jnp.concatenate([d0, d[:, T:], d2], axis=1)))
            head(h)
        dscores(jnp.minimum(n + 2, last), n % 2)
        sc = DH ** -0.5
        dqkv[g, b + 2] = (jnp.concatenate(dqs, axis=0) * sc).astype(bf16)
        for t, parts, c in ((1, dks, 1.0 / LOG2E), (2, dvs, None)):
            d3 = jnp.concatenate(parts, axis=0)
            if c is not None:
                d3 = d3 * c
            dqkv[t * NG + g, b] = (acc_v[t - 1, g, 0] + d3[:, :T]).astype(bf16)
            acc_v[t - 1, g, 0] = acc_v[t - 1, g, 1] + d3[:, T:2 * T]
            acc_v[t - 1, g, 1] = d3[:, 2 * T:]
        return 0
    outs[0].wait()
    xin = pltpu.make_async_copy(x_h, x_v, sem.at[7])
    xin.start()
    acc_v[...] = jnp.zeros(acc_v.shape, f32)
    jax.lax.fori_loop(0, NB * NG, att_bwd, 0, unroll=16)

    for t in (1, 2):
        for g in range(NG):
            for j in range(2):
                dqkv[t * NG + g, NB + j] = acc_v[t - 1, g, j].astype(bf16)

    xin.wait()

    def dx_body(i, _):
        rows = pl.ds(pl.multiple_of(i * RB, RB), RB)
        dT = jnp.concatenate([jnp.concatenate(
            [dqkv[a, i * (RB // T) + j + 2] for j in range(RB // T)], axis=1)
            for a in range(3 * NG)], axis=0)
        dy = _nn(wqkv_v[...], dT).T
        y, r = _ln(x_v[rows].astype(f32))
        go_v[rows] = (h_v[rows] + _ln_bwd(dy, y, r)).astype(bf16)
        return 0
    jax.lax.fori_loop(0, S // RB, dx_body, 0, unroll=4)
    outs[1].start()
    fin = []
    for j, (t, c0, nc) in enumerate(((0, 0, D), (1, 0, D), (2, 0, 3 * T), (2, 3 * T, T))):
        gs = range(c0 // T, (c0 + nc) // T)
        dT = jnp.concatenate([jnp.concatenate(
            [dqkv[t * NG + g, k + 2] for k in range(NB)], axis=1) for g in gs], axis=0)
        cols = pl.ds(t * D + c0, nc)
        wqkv_v[:, cols] = _nt(ln1t[...], dT).astype(bf16)
        fin.append(pltpu.make_async_copy(wqkv_v.at[:, cols], dwqkv_h.at[:, cols], sem.at[10 + j]))
        fin[-1].start()
    for c in [outs[1]] + outs[2:] + fin:
        c.wait()


@jax.jit
def pallas_sequential_preLN__sliding_block__glu_gated_glu__prompt_kernel(
    A_x, A_wqkv, A_wo, B_x, B_w_gate, B_w_up, B_w_down, grad_out,
):
    V = pltpu.VMEM
    sds = jax.ShapeDtypeStruct
    outs = pl.pallas_call(
        _kernel,
        in_specs=[pl.BlockSpec(memory_space=pl.ANY)] * 7,
        out_specs=[pl.BlockSpec(memory_space=pl.ANY)] * 7,
        out_shape=[sds((S, D), bf16), sds((S, D), bf16), sds((D, 3 * D), bf16), sds((D, D), bf16),
                   sds((F, D), bf16), sds((F, D), bf16), sds((F, D), bf16)],
        scratch_shapes=[
            V((S, D), bf16), V((S, D), bf16), V((D, 3 * D), bf16), V((D, D), bf16),
            V((F, D), bf16), V((F, D), bf16), V((F, D), bf16),
            V((D, S), bf16), V((NG, NB, T, T), bf16), V((NG, NB, T, T), bf16), V((NG, NB + 2, T, T), bf16),
            V((NG, NB + 2, T, T), bf16), V((NG, S + 2 * T, T), bf16),
            V((NG, NB, T, T), bf16), V((NG, NB, HG, T), f32), V((NB * NG, HG, T, 2 * T), bf16), V((S, D), f32),
            V((D, S), bf16), V((D, S), bf16), V((S, F), bf16), V((S, F), bf16), V((S, F), bf16),
            V((3 * NG, NB + 2, T, T), bf16), V((2, NG, 2, T, T), f32),
            V((HG, 2 * T, T), f32), V((HG, 1, T), f32), V((2, T, T), bf16), V((HG, T, 2 * T), f32), V((4, T, T), bf16),
            V((HT // 2, T), jnp.uint32), V((T // 2, T), jnp.uint32), V((T // 2, T), jnp.uint32),
            V((HG + 2, HT // 2, T), jnp.uint32),
            pltpu.SemaphoreType.DMA((14,)),
        ],
        compiler_params=pltpu.CompilerParams(vmem_limit_bytes=127 * 2**20),
    )(A_x.reshape(S, D), A_wqkv, A_wo, B_w_gate.T, B_w_up.T, B_w_down, grad_out.reshape(S, D))
    return (outs[0].reshape(1, S, D), outs[1].reshape(1, S, D), outs[2], outs[3], outs[4].T, outs[5].T, outs[6])
```
